```python
import os as _os
_os.environ.setdefault('JAX_PLATFORMS', 'cpu')
import jax
import jax.numpy as jnp

def _softmax(x, axis=-1):
    return jax.nn.softmax(x, axis=axis)

def _gelu(x):
    return jax.nn.gelu(x, approximate=True)

def _silu(x):
    return jax.nn.silu(x)

def _sigmoid(x):
    return jax.nn.sigmoid(x)

def _layernorm(x, axis=-1, eps=1e-05):
    m = jnp.mean(x, axis=axis, keepdims=True)
    v = jnp.var(x, axis=axis, keepdims=True)
    return (x - m) / jnp.sqrt(v + eps)

def _scatter_add(tgt, idx, src, axis=0):
    return tgt.at[idx].add(src)

def _segment_sum(src, seg, n):
    return jax.ops.segment_sum(src, seg, n)

class _Rng:

    def __init__(self, key):
        self._k = key

    def _next(self):
        self._k, sub = jax.random.split(self._k)
        return sub

    def normal(self, shape):
        return jax.random.normal(self._next(), shape, dtype=jnp.bfloat16)

    def randint(self, lo, hi, shape):
        return jax.random.randint(self._next(), shape, lo, hi, dtype=jnp.int32)

    def uniform(self, shape, lo=0.0, hi=1.0):
        return jax.random.uniform(self._next(), shape, jnp.bfloat16, lo, hi)

    def permutation(self, n):
        return jax.random.permutation(self._next(), n)
kernel_name = 'standalone__autoregressive_conv_wavenet__speech'

def setup_inputs():
    _rng = _Rng(jax.random.key(int.from_bytes(__import__("os").urandom(4), "little")))
    _w = lambda a: (lambda t: t.astype(jnp.bfloat16) if jnp.issubdtype(t.dtype, jnp.floating) else t)(jnp.asarray(a))
    B, T, D, K = (2, 4000, 512, 31)
    return {'x': _w((lambda *s: _rng.normal(s) * 0.05)(B, T, D)), 'w': _w((lambda *s: _rng.normal(s) * 0.05)(K, D, 2 * D)), 'w_o': _w((lambda *s: _rng.normal(s) * 0.05)(D, D))}

def reference(x, w, w_o):
    B, T, D = x.shape
    K = w.shape[0]
    dil = 2
    pad = (K - 1) * dil
    xp = jnp.pad(x, ((0, 0), (pad, 0), (0, 0)))
    h = jnp.einsum('btc,cd->btd', xp[:, pad:pad + T, :], w[0])
    for i in range(1, K):
        off = pad - i * dil
        h = h + jnp.einsum('btc,cd->btd', xp[:, off:off + T, :], w[i])
    f = h[..., :D].copy()
    g = h[..., D:].copy()
    z = jnp.tanh(f) * _sigmoid(g)
    return z @ w_o
```

```python
import jax, jax.numpy as jnp
import jax.experimental.pallas as pl
import jax.experimental.pallas.tpu as pltpu

TT = 800
HALO = 64

def _kernel(x_hbm, w_ref, wo_ref, o_ref, xw_ref, sem, *, TT, HALO, D, K):
    b = pl.program_id(0); t = pl.program_id(1)
    t0 = t * TT

    @pl.when(t == 0)
    def _():
        xw_ref[0:HALO, :] = jnp.zeros((HALO, D), xw_ref.dtype)
        cp = pltpu.make_async_copy(x_hbm.at[b, pl.ds(0, TT)], xw_ref.at[pl.ds(HALO, TT)], sem)
        cp.start(); cp.wait()

    @pl.when(t > 0)
    def _():
        cp = pltpu.make_async_copy(x_hbm.at[b, pl.ds(t0 - HALO, TT + HALO)], xw_ref, sem)
        cp.start(); cp.wait()

    h = None
    for i in range(K):
        off = HALO - 2 * i
        lhs = xw_ref[pl.ds(off, TT), :]
        p = jnp.dot(lhs, w_ref[i], preferred_element_type=jnp.float32)
        h = p if h is None else h + p
    f = h[:, :D]; g = h[:, D:]
    z = (jnp.tanh(f) * jax.nn.sigmoid(g)).astype(jnp.bfloat16)
    o_ref[0] = jnp.dot(z, wo_ref[...], preferred_element_type=jnp.float32).astype(o_ref.dtype)


@jax.jit
def pallas_standalone__autoregressive_conv_wavenet__speech_kernel(x, w, w_o):
    B, T, D = x.shape
    K = w.shape[0]
    import functools
    kern = functools.partial(_kernel, TT=TT, HALO=HALO, D=D, K=K)
    return pl.pallas_call(
        kern,
        grid_spec=pltpu.PrefetchScalarGridSpec(
            num_scalar_prefetch=0,
            grid=(B, T // TT),
            in_specs=[
                pl.BlockSpec(memory_space=pl.ANY),
                pl.BlockSpec((K, D, 2 * D), lambda b, t: (0, 0, 0), pipeline_mode=pl.Buffered(1)),
                pl.BlockSpec((D, D), lambda b, t: (0, 0), pipeline_mode=pl.Buffered(1)),
            ],
            out_specs=pl.BlockSpec((1, TT, D), lambda b, t: (b, t, 0)),
            scratch_shapes=[
                pltpu.VMEM((TT + HALO, D), jnp.bfloat16),
                pltpu.SemaphoreType.DMA,
            ],
        ),
        out_shape=jax.ShapeDtypeStruct((B, T, D), jnp.bfloat16),
        compiler_params=pltpu.CompilerParams(
            dimension_semantics=("arbitrary", "arbitrary"),
            vmem_limit_bytes=110 * 1024 * 1024),
    )(x, w, w_o)
```

```python
import functools
import jax, jax.numpy as jnp
import jax.experimental.pallas as pl
import jax.experimental.pallas.tpu as pltpu

TT = 2000
WLOOK = 4
HALO = 72
LO = 16

def _kernel(x_hbm, w_hbm, wo_ref, o_ref, xs_ref, xc_ref, w_vmem, acc_ref, x_sem, w_sems,
            *, TT, D, K, NB, NT):
    b = pl.program_id(0); t = pl.program_id(1)
    step = b * NT + t
    last = NB * NT - 1
    L = TT + HALO - LO

    def xcopy(bb, tt):
        t0n = tt * TT
        c0 = pltpu.make_async_copy(x_hbm.at[bb, pl.ds(0, TT)],
                                   xs_ref.at[pl.ds(HALO, TT)], x_sem)
        c1 = pltpu.make_async_copy(x_hbm.at[bb, pl.ds(pl.multiple_of(jnp.maximum(t0n - HALO, 0), 8), TT + HALO)],
                                   xs_ref, x_sem)
        return c0, c1

    def wcopy(k):
        return pltpu.make_async_copy(w_hbm.at[k], w_vmem.at[k], w_sems.at[k])

    @pl.when(step == 0)
    def _():
        c0, c1 = xcopy(b, t)
        c0.start()
        for k in range(WLOOK):
            wcopy(k).start()

    c0, c1 = xcopy(b, t)
    @pl.when(t == 0)
    def _():
        c0.wait()
        xs_ref[0:HALO, :] = jnp.zeros((HALO, D), xs_ref.dtype)
    @pl.when(t > 0)
    def _():
        c1.wait()

    @pl.when(pl.program_id(1) < NT)
    def _cps():
        for r in range(4):
            xc_ref[r, LO:LO + L, :] = xs_ref[pl.ds(LO - 2 * r, L), :]

    @pl.when(step < last)
    def _():
        tn = t + 1
        wrap = tn == NT
        tn2 = jnp.where(wrap, 0, tn)
        bn2 = jnp.where(wrap, b + 1, b)
        n0, n1 = xcopy(bn2, tn2)
        @pl.when(tn2 == 0)
        def _():
            n0.start()
        @pl.when(tn2 > 0)
        def _():
            n1.start()

    acc_ref[...] = jnp.zeros(acc_ref.shape, acc_ref.dtype)
    for r in range(4):
        nm = (K - r + 3) // 4
        def body(m, carry, r=r):
            k = 4 * m + r
            off = pl.multiple_of(HALO - 8 * m, 8)
            @pl.when(step == 0)
            def _():
                wcopy(k).wait()
                @pl.when(k + WLOOK < K)
                def _():
                    wcopy(jnp.minimum(k + WLOOK, K - 1)).start()
            lhs = xc_ref[r, pl.ds(off, TT), :]
            acc_ref[...] += jnp.dot(lhs, w_vmem[k], preferred_element_type=jnp.float32)
            return carry
        jax.lax.fori_loop(0, nm, body, 0)

    h = acc_ref[...]
    f = h[:, :D]; g = h[:, D:]
    z = (jnp.tanh(f) * jax.nn.sigmoid(g)).astype(jnp.bfloat16)
    o_ref[0] = jnp.dot(z, wo_ref[...], preferred_element_type=jnp.float32).astype(o_ref.dtype)


@jax.jit
def pallas_standalone__autoregressive_conv_wavenet__speech_kernel(x, w, w_o):
    B, T, D = x.shape
    K = w.shape[0]
    assert T % TT == 0
    NT = T // TT
    kern = functools.partial(_kernel, TT=TT, D=D, K=K, NB=B, NT=NT)
    return pl.pallas_call(
        kern,
        grid_spec=pltpu.PrefetchScalarGridSpec(
            num_scalar_prefetch=0,
            grid=(B, NT),
            in_specs=[
                pl.BlockSpec(memory_space=pl.ANY),
                pl.BlockSpec(memory_space=pl.ANY),
                pl.BlockSpec((D, D), lambda b, t: (0, 0), pipeline_mode=pl.Buffered(1)),
            ],
            out_specs=pl.BlockSpec((1, TT, D), lambda b, t: (b, t, 0)),
            scratch_shapes=[
                pltpu.VMEM((TT + HALO, D), jnp.bfloat16),
                pltpu.VMEM((4, TT + HALO, D), jnp.bfloat16),
                pltpu.VMEM((K, D, 2 * D), jnp.bfloat16),
                pltpu.VMEM((TT, 2 * D), jnp.float32),
                pltpu.SemaphoreType.DMA,
                pltpu.SemaphoreType.DMA((K,)),
            ],
        ),
        out_shape=jax.ShapeDtypeStruct((B, T, D), jnp.bfloat16),
        compiler_params=pltpu.CompilerParams(
            dimension_semantics=("arbitrary", "arbitrary"),
            vmem_limit_bytes=120 * 1024 * 1024),
    )(x, w, w_o)
```

```python
import functools
import jax, jax.numpy as jnp
import jax.experimental.pallas as pl
import jax.experimental.pallas.tpu as pltpu

TT = 2000
WLOOK = 4
HALO = 72
LO = 16

def _kernel(x_hbm, w_hbm, wo_ref, o_ref, xs_ref, xc_ref, w_vmem, acc_ref, x_sem, w_sems,
            *, TT, D, K, NB, NT):
    b = pl.program_id(0); t = pl.program_id(1)
    step = b * NT + t
    last = NB * NT - 1
    L = TT + HALO - LO

    def xcopy(bb, tt):
        t0n = tt * TT
        c0 = pltpu.make_async_copy(x_hbm.at[bb, pl.ds(0, TT)],
                                   xs_ref.at[pl.ds(HALO, TT)], x_sem)
        c1 = pltpu.make_async_copy(x_hbm.at[bb, pl.ds(pl.multiple_of(jnp.maximum(t0n - HALO, 0), 8), TT + HALO)],
                                   xs_ref, x_sem)
        return c0, c1

    def wcopy(k):
        return pltpu.make_async_copy(w_hbm.at[k], w_vmem.at[k], w_sems.at[k])

    @pl.when(step == 0)
    def _():
        c0, c1 = xcopy(b, t)
        c0.start()
        for k in range(WLOOK):
            wcopy(k).start()

    c0, c1 = xcopy(b, t)
    @pl.when(t == 0)
    def _():
        c0.wait()
        xs_ref[0:HALO, :] = jnp.zeros((HALO, D), xs_ref.dtype)
    @pl.when(t > 0)
    def _():
        c1.wait()

    @pl.when(pl.program_id(1) < NT)
    def _cps():
        for r in range(1, 4):
            xc_ref[r, LO:LO + L, :] = xs_ref[pl.ds(LO - 2 * r, L), :]

    @pl.when(step == 0)
    def _():
        acc_ref[...] = jnp.zeros(acc_ref.shape, acc_ref.dtype)
    for r in range(4):
        nm = (K - r + 3) // 4
        def body(m, carry, r=r):
            k = 4 * m + r
            off = pl.multiple_of(HALO - 8 * m, 8)
            @pl.when(step == 0)
            def _():
                wcopy(k).wait()
                @pl.when(k + WLOOK < K)
                def _():
                    wcopy(jnp.minimum(k + WLOOK, K - 1)).start()
            lhs = (xs_ref if r == 0 else xc_ref.at[r])[pl.ds(off, TT), :]
            acc_ref[...] += jnp.dot(lhs, w_vmem[k], preferred_element_type=jnp.float32)
            return carry
        jax.lax.fori_loop(0, nm, body, 0)
        if r == 0:
            @pl.when(step < last)
            def _():
                tn = t + 1
                wrap = tn == NT
                tn2 = jnp.where(wrap, 0, tn)
                bn2 = jnp.where(wrap, b + 1, b)
                n0, n1 = xcopy(bn2, tn2)
                @pl.when(tn2 == 0)
                def _():
                    n0.start()
                @pl.when(tn2 > 0)
                def _():
                    n1.start()

    h = acc_ref[...]
    acc_ref[...] = jnp.zeros(acc_ref.shape, acc_ref.dtype)
    f = h[:, :D]; g = h[:, D:]
    z = (jnp.tanh(f) * (0.5 * jnp.tanh(0.5 * g) + 0.5)).astype(jnp.bfloat16)
    o_ref[0] = jnp.dot(z, wo_ref[...], preferred_element_type=jnp.float32).astype(o_ref.dtype)


@jax.jit
def pallas_standalone__autoregressive_conv_wavenet__speech_kernel(x, w, w_o):
    B, T, D = x.shape
    K = w.shape[0]
    assert T % TT == 0
    NT = T // TT
    kern = functools.partial(_kernel, TT=TT, D=D, K=K, NB=B, NT=NT)
    return pl.pallas_call(
        kern,
        grid_spec=pltpu.PrefetchScalarGridSpec(
            num_scalar_prefetch=0,
            grid=(B, NT),
            in_specs=[
                pl.BlockSpec(memory_space=pl.ANY),
                pl.BlockSpec(memory_space=pl.ANY),
                pl.BlockSpec((D, D), lambda b, t: (0, 0), pipeline_mode=pl.Buffered(1)),
            ],
            out_specs=pl.BlockSpec((1, TT, D), lambda b, t: (b, t, 0)),
            scratch_shapes=[
                pltpu.VMEM((TT + HALO, D), jnp.bfloat16),
                pltpu.VMEM((4, TT + HALO, D), jnp.bfloat16),
                pltpu.VMEM((K, D, 2 * D), jnp.bfloat16),
                pltpu.VMEM((TT, 2 * D), jnp.float32),
                pltpu.SemaphoreType.DMA,
                pltpu.SemaphoreType.DMA((K,)),
            ],
        ),
        out_shape=jax.ShapeDtypeStruct((B, T, D), jnp.bfloat16),
        compiler_params=pltpu.CompilerParams(
            dimension_semantics=("arbitrary", "arbitrary"),
            vmem_limit_bytes=120 * 1024 * 1024),
    )(x, w, w_o)
```
